```python
import jax
import jax.numpy as jnp

def _softmax(x, axis=-1):
    return jax.nn.softmax(x, axis=axis)

def _gelu(x):
    return jax.nn.gelu(x, approximate=True)

def _silu(x):
    return jax.nn.silu(x)

def _sigmoid(x):
    return jax.nn.sigmoid(x)

def _layernorm(x, axis=-1, eps=1e-05):
    m = jnp.mean(x, axis=axis, keepdims=True)
    v = jnp.var(x, axis=axis, keepdims=True)
    return (x - m) / jnp.sqrt(v + eps)

def _scatter_add(tgt, idx, src, axis=0):
    return tgt.at[idx].add(src)

def _segment_sum(src, seg, n):
    return jax.ops.segment_sum(src, seg, n)

class _Rng:

    def __init__(self, key):
        self._k = key

    def _next(self):
        self._k, sub = jax.random.split(self._k)
        return sub

    def normal(self, shape):
        return jax.random.normal(self._next(), shape, dtype=jnp.bfloat16)

    def randint(self, lo, hi, shape):
        return jax.random.randint(self._next(), shape, lo, hi, dtype=jnp.int32)

    def uniform(self, shape, lo=0.0, hi=1.0):
        return jax.random.uniform(self._next(), shape, jnp.bfloat16, lo, hi)

    def permutation(self, n):
        return jax.random.permutation(self._next(), n)
kernel_name = 'adaLN_cond__sliding_local_dilated__mixer_s_mlp__prompt'

def setup_inputs():
    _rng = _Rng(jax.random.key(int.from_bytes(__import__("os").urandom(4), "little")))
    _w = lambda a: (lambda t: t.astype(jnp.bfloat16) if jnp.issubdtype(t.dtype, jnp.floating) else t)(jnp.asarray(a))

    def _A_setup():
        B, S, D = (1, 2048, 1024)
        return {'x': _w((lambda *s: _rng.normal(s) * 0.05)(B, S, D)), 'wqkv': _w((lambda *s: _rng.normal(s) * 0.05)(D, 3 * D)), 'wo': _w((lambda *s: _rng.normal(s) * 0.05)(D, D))}
    _A_in = _A_setup()

    def _B_setup():
        B, S, D, F = (1, 2048, 1024, 3584)
        return {'x': _w((lambda *s: _rng.normal(s) * 0.05)(B, S, D)), 'w1': _w((lambda *s: _rng.normal(s) * 0.05)(D, D) * D ** (-0.5)), 'w2': _w((lambda *s: _rng.normal(s) * 0.05)(D, D) * D ** (-0.5)), 'w3': _w((lambda *s: _rng.normal(s) * 0.05)(D, F) * D ** (-0.5)), 'w4': _w((lambda *s: _rng.normal(s) * 0.05)(F, D) * F ** (-0.5))}
    _B_in = _B_setup()
    return {'A_x': _A_in['x'], 'A_wqkv': _A_in['wqkv'], 'A_wo': _A_in['wo'], 'B_x': _B_in['x'], 'B_w1': _B_in['w1'], 'B_w2': _B_in['w2'], 'B_w3': _B_in['w3'], 'B_w4': _B_in['w4'], 'c': _w((lambda *s: _rng.normal(s) * 0.05)(1, 1024)), 'w_mod': _w((lambda *s: _rng.normal(s) * 0.05)(1024, 6 * 1024) * 1024 ** (-0.5))}

def reference(A_x, A_wqkv, A_wo, B_x, B_w1, B_w2, B_w3, B_w4, c, w_mod):

    def _A_ref(x, wqkv, wo):
        B, S, D = x.shape
        H = 32
        Dh = D // H
        W, dil = (8, 2)
        qkv = (lambda x, *d: x.transpose(*d))((x @ wqkv).reshape(B, S, 3, H, Dh), 2, 0, 3, 1, 4)
        q, k, v = (qkv[0], qkv[1], qkv[2])
        scale = Dh ** (-0.5)
        pos = jnp.arange(S)
        off = jnp.arange(W) * dil
        idx = pos[:, None] - off[None, :]
        mask = idx >= 0
        idx_c = jnp.where(mask, idx, 0).reshape(-1)
        kg = k[:, :, idx_c, :].reshape(B, H, S, W, Dh)
        vg = v[:, :, idx_c, :].reshape(B, H, S, W, Dh)
        logits = jnp.einsum('bhsd,bhswd->bhsw', q, kg) * scale
        logits = jnp.where(mask[None, None, :, :], logits, -1000000000.0)
        attn = _softmax(logits, axis=-1)
        o = jnp.einsum('bhsw,bhswd->bhsd', attn, vg)
        return (lambda x, *d: x.transpose(*d))(o, 0, 2, 1, 3).reshape(B, S, D) @ wo

    def _B_ref(x, w1, w2, w3, w4):
        B, S, D = x.shape
        h = _gelu(_layernorm(x, axis=-1) @ w1)
        c = D // 4
        g0 = jnp.pad(h[:, :, 0 * c:1 * c], ((0, 0), (1, 0), (0, 0)))[:, :S, :]
        g1 = jnp.pad(h[:, :, 1 * c:2 * c], ((0, 0), (0, 1), (0, 0)))[:, 1:, :]
        g2 = jnp.pad(h[:, :, 2 * c:3 * c], ((0, 0), (2, 0), (0, 0)))[:, :S, :]
        g3 = jnp.pad(h[:, :, 3 * c:], ((0, 0), (0, 2), (0, 0)))[:, 2:, :]
        hs = jnp.concatenate([g0, g1, g2, g3], axis=-1) @ w2
        x1 = x + hs
        h2 = _gelu(_layernorm(x1, axis=-1) @ w3) @ w4
        return x1 + h2
    x = A_x
    mod = (_silu(c) @ w_mod).reshape(c.shape[0], 6, 1, -1)
    sa, ca, ga, sb, cb, gb = (mod[:, 0].copy(), mod[:, 1].copy(), mod[:, 2].copy(), mod[:, 3].copy(), mod[:, 4].copy(), mod[:, 5].copy())
    h = _layernorm(x, axis=-1) * (1 + ca) + sa
    x = x + ga * _A_ref(h, A_wqkv, A_wo)
    h = _layernorm(x, axis=-1) * (1 + cb) + sb
    x = x + gb * _B_ref(h, B_w1, B_w2, B_w3, B_w4)
    return x
```

```python
import functools
import math

import jax
import jax.numpy as jnp
import jax.experimental.pallas as pl
import jax.experimental.pallas.tpu as pltpu

S, D, F = 2048, 1024, 3584
H, DH, W, DIL = 32, 32, 8, 2
T = 512
NB = S // T
HALO = 16
FC = 512
NF = F // FC
RC = 64
NCB = D // 128
BF, F32 = jnp.bfloat16, jnp.float32
EPS = 1e-5


def _ln(x):
    m = jnp.mean(x, axis=-1, keepdims=True)
    xc = x - m
    v = jnp.mean(xc * xc, axis=-1, keepdims=True)
    return xc * jax.lax.rsqrt(v + EPS)


def _gelu(x):
    c = math.sqrt(2.0 / math.pi)
    t = jnp.tanh(x * (c + (c * 0.044715) * (x * x)))
    hx = 0.5 * x
    return hx + hx * t


def _dot(a, b):
    return jnp.dot(a, b, preferred_element_type=F32)


def _permute_cols(w_ref, r0, nr, c0):
    blk = [pltpu.bitcast(w_ref[pl.ds(r0, nr), c0 + b * 128:c0 + (b + 1) * 128], jnp.uint32)
           for b in range(NCB)]
    lane = jax.lax.broadcasted_iota(jnp.int32, blk[0].shape, 1)
    src = (lane & 3) * 32 + (lane & 28) + (lane >> 5)
    blk = [jnp.take_along_axis(x, src, axis=1) for x in blk]
    for t in range(3):
        sh = 4 << t
        low = (lane & sh) == 0
        for b in range(NCB):
            if b & (1 << t):
                continue
            lo, hi = blk[b], blk[b | (1 << t)]
            blk[b] = jnp.where(low, lo, pltpu.roll(hi, sh, 1))
            blk[b | (1 << t)] = jnp.where(low, pltpu.roll(lo, 128 - sh, 1), hi)
    for b in range(NCB):
        w_ref[pl.ds(r0, nr), c0 + b * 128:c0 + (b + 1) * 128] = pltpu.bitcast(blk[b], BF)


def _kernel(x_h, c_ref, wmod_h, wqkv_h, wo_h, w1_h, w2_h, w3_h, w4_h, out_h,
            xv, wmod, wqkv, wo, w1, w2, w3, w4, wo_tmp, mod, qbuf, kbuf, vbuf, obuf,
            xa, hb, h1, ostage, sems, osem):
    def cols(src, dst, c0, n):
        return src.at[:, pl.ds(c0, n)], dst.at[:, pl.ds(c0, n)]

    def rows(src, dst, r0, n):
        return src.at[pl.ds(r0, n)], dst.at[pl.ds(r0, n)]

    pairs = dict(
        wq=cols(wqkv_h, wqkv, 0, D), mod0=cols(wmod_h, wmod, 0, 2 * D), x0=rows(x_h, xv, 0, T),
        wk=cols(wqkv_h, wqkv, D, D), wv=cols(wqkv_h, wqkv, 2 * D, D),
        mod1=cols(wmod_h, wmod, 2 * D, 4 * D), wo=(wo_h, wo), w1=(w1_h, w1),
        x1=rows(x_h, xv, T, S - T), w2=(w2_h, w2), w3=(w3_h, w3), w4=(w4_h, w4))
    cp = {k: pltpu.make_async_copy(s_, d_, sems.at[n]) for n, (k, (s_, d_)) in enumerate(pairs.items())}

    def silu_c():
        cv = c_ref[...].astype(F32)
        s = (cv * jax.nn.sigmoid(cv)).astype(BF)
        return jnp.broadcast_to(s, (16, D))

    def perm(j):
        for r0 in range(0, D, 64):
            _permute_cols(wqkv, r0, 64, j * D)

    def a_qkv(blk):
        x = xv[blk * T:(blk + 1) * T, :].astype(F32)
        h = (_ln(x) * (1.0 + mod[1:2, :]) + mod[0:1, :]).astype(BF)
        q = _dot(h, wqkv[:, 0:D])
        for b in range(NCB):
            qbuf[b] = q[:, b * 128:(b + 1) * 128] * (DH ** -0.5)
        if blk == 0:
            cp["wk"].wait()
            perm(1)
        k = _dot(h, wqkv[:, D:2 * D])
        for b in range(NCB):
            kbuf[b, HALO:, :] = k[:, b * 128:(b + 1) * 128]
        if blk == 0:
            cp["wv"].wait()
            perm(2)
        v = _dot(h, wqkv[:, 2 * D:3 * D])
        for b in range(NCB):
            vbuf[b, HALO:, :] = v[:, b * 128:(b + 1) * 128]

    def a_attn(r0, first):
        q = [qbuf[b, r0:r0 + RC, :] for b in range(NCB)]
        ls = []
        for w in range(W):
            o = HALO + r0 - DIL * w
            acc = None
            for b in range(NCB):
                p = q[b] * kbuf[b, o:o + RC, :]
                acc = p if acc is None else acc + p
            acc = acc + pltpu.roll(acc, 64, 1)
            acc = acc + pltpu.roll(acc, 32, 1)
            if first and r0 < DIL * w:
                pos = jax.lax.broadcasted_iota(jnp.int32, acc.shape, 0) + r0
                acc = jnp.where(pos >= DIL * w, acc, -1e9)
            ls.append(acc)
        m = functools.reduce(jnp.maximum, ls)
        es = [jnp.exp(l - m) for l in ls]
        inv = 1.0 / functools.reduce(lambda a, b: a + b, es)
        ps = [e * inv for e in es]
        for b in range(NCB):
            acc = None
            for w in range(W):
                o = HALO + r0 - DIL * w
                p = ps[w] * vbuf[b, o:o + RC, :]
                acc = p if acc is None else acc + p
            obuf[r0:r0 + RC, b * 128:(b + 1) * 128] = acc.astype(BF)

    def a_tail(slot):
        for b in range(NCB):
            kbuf[b, 0:HALO, :] = kbuf[b, T:T + HALO, :]
            vbuf[b, 0:HALO, :] = vbuf[b, T:T + HALO, :]
        xn = xv[slot * T:(slot + 1) * T, :].astype(F32) + mod[2:3, :] * _dot(obuf[...], wo[...])
        h = _ln(xn) * (1.0 + mod[4:5, :]) + mod[3:4, :]
        r = HALO + slot * T
        xa[pl.ds(r, T), :] = xn
        hb[pl.ds(r, T), :] = h
        g = _gelu(_dot(_ln(h).astype(BF), w1[...]))
        r1 = 2 * HALO + slot * T
        for b in range(NCB):
            h1[b, pl.ds(r1, T), :] = g[:, b * 128:(b + 1) * 128]

    def b_head(blk, n):
        r = blk * T
        parts = []
        for b in range(NCB):
            sh = (1, -1, 2, -2)[b // 2]
            parts.append(h1[b, pl.ds(r + HALO - sh, n), :].astype(BF))
        hs = _dot(jnp.concatenate(parts, axis=1), w2[...])
        x1 = hb[pl.ds(r, n), :] + hs
        return x1, _ln(x1).astype(BF)

    def b_chunk(acc, ln1, f):
        g = _gelu(_dot(ln1, w3[:, f * FC:(f + 1) * FC])).astype(BF)
        return acc + _dot(g, w4[f * FC:(f + 1) * FC, :])

    def b_tail(blk, n, acc):
        r = blk * T
        y = xa[pl.ds(r, n), :] + mod[5:6, :] * acc
        ostage[pl.ds(r, n), :] = y.astype(BF)

    def out_copy(blk):
        lo = max(blk * T - HALO, 0)
        hi = S if blk == NB - 1 else (blk + 1) * T - HALO
        return pltpu.make_async_copy(ostage.at[pl.ds(lo + HALO, hi - lo)], out_h.at[pl.ds(lo, hi - lo)], osem.at[blk])

    nrc = T // RC

    for c_ in cp.values():
        c_.start()
    xa[0:HALO, :] = jnp.zeros((HALO, D), F32)
    hb[0:HALO, :] = jnp.zeros((HALO, D), F32)
    for b in range(NCB):
        h1[b, 0:2 * HALO, :] = jnp.zeros((2 * HALO, 128), F32)
        h1[b, S + 2 * HALO:, :] = jnp.zeros((HALO, 128), F32)
        kbuf[b, 0:HALO, :] = jnp.zeros((HALO, 128), F32)
    sc = silu_c()
    cp["wq"].wait()
    perm(0)
    cp["mod0"].wait()
    for j in range(2):
        mod[j:j + 1, :] = _dot(sc, wmod[:, j * D:(j + 1) * D])[0:1, :]
    cp["x0"].wait()
    a_qkv(0)
    for b in range(NCB):
        vbuf[b, 0:HALO, :] = jnp.broadcast_to(vbuf[b, HALO:HALO + 1, :], (HALO, 128))
    cp["mod1"].wait()
    cp["wo"].wait()
    for j in range(2, 6):
        mod[j:j + 1, :] = _dot(sc, wmod[:, j * D:(j + 1) * D])[0:1, :]
    for b in range(NCB):
        wo_tmp[b] = wo[:, b * 128:(b + 1) * 128].astype(F32)
    for d in range(DH):
        rws = jnp.concatenate([wo_tmp[b, pl.ds(d, H, stride=DH), :] for b in range(NCB)], axis=1)
        wo[d * H:(d + 1) * H, :] = rws.astype(BF)
    for c in range(nrc):
        a_attn(c * RC, True)
    cp["w1"].wait()
    a_tail(0)
    for k in ("x1", "w2", "w3", "w4"):
        cp[k].wait()

    for i in range(1, NB):
        a_qkv(i)
        x1, ln1 = b_head(i - 1, T)
        acc = x1
        for f in range(NF):
            acc = b_chunk(acc, ln1, f)
            for c in range(f * nrc // NF, (f + 1) * nrc // NF):
                a_attn(c * RC, False)
        b_tail(i - 1, T, acc)
        out_copy(i - 1).start()
        a_tail(i)

    n = T + HALO
    x1, ln1 = b_head(NB - 1, n)
    acc = x1
    for f in range(NF):
        acc = b_chunk(acc, ln1, f)
    b_tail(NB - 1, n, acc)
    out_copy(NB - 1).start()
    for blk in range(NB):
        out_copy(blk).wait()


@jax.jit
def pallas_adaLN_cond__sliding_local_dilated__mixer_s_mlp__prompt_kernel(
    A_x: jax.Array,
    A_wqkv: jax.Array,
    A_wo: jax.Array,
    B_x: jax.Array,
    B_w1: jax.Array,
    B_w2: jax.Array,
    B_w3: jax.Array,
    B_w4: jax.Array,
    c: jax.Array,
    w_mod: jax.Array,
):
    del B_x
    hbm = pl.BlockSpec(memory_space=pl.ANY)
    out = pl.pallas_call(
        _kernel,
        in_specs=[
            hbm,
            pl.BlockSpec(memory_space=pltpu.VMEM),
        ] + [hbm] * 7,
        out_specs=hbm,
        out_shape=jax.ShapeDtypeStruct((S, D), BF),
        scratch_shapes=[
            pltpu.VMEM((S, D), BF),
            pltpu.VMEM((D, 6 * D), BF),
            pltpu.VMEM((D, 3 * D), BF),
            pltpu.VMEM((D, D), BF),
            pltpu.VMEM((D, D), BF),
            pltpu.VMEM((D, D), BF),
            pltpu.VMEM((D, F), BF),
            pltpu.VMEM((F, D), BF),
            pltpu.VMEM((NCB, D, 128), F32),
            pltpu.VMEM((8, D), F32),
            pltpu.VMEM((NCB, T, 128), F32),
            pltpu.VMEM((NCB, T + HALO, 128), F32),
            pltpu.VMEM((NCB, T + HALO, 128), F32),
            pltpu.VMEM((T, D), BF),
            pltpu.VMEM((S + HALO, D), F32),
            pltpu.VMEM((S + HALO, D), F32),
            pltpu.VMEM((NCB, S + 3 * HALO, 128), F32),
            pltpu.VMEM((S + HALO, D), BF),
            pltpu.SemaphoreType.DMA((12,)),
            pltpu.SemaphoreType.DMA((NB,)),
        ],
        compiler_params=pltpu.CompilerParams(
            vmem_limit_bytes=120 * 1024 * 1024,
        ),
    )(A_x.reshape(S, D), c, w_mod, A_wqkv, A_wo, B_w1, B_w2, B_w3, B_w4)
    return out.reshape(1, S, D)
```

```python
import functools
import math

import jax
import jax.numpy as jnp
import jax.experimental.pallas as pl
import jax.experimental.pallas.tpu as pltpu

S, D, F = 2048, 1024, 3584
H, DH, W, DIL = 32, 32, 8, 2
T = 512
NB = S // T
HALO = 16
FC = 512
NF = F // FC
RC = 64
NCB = D // 128
BF, F32 = jnp.bfloat16, jnp.float32
EPS = 1e-5


def _ln(x):
    m = jnp.mean(x, axis=-1, keepdims=True)
    xc = x - m
    v = jnp.mean(xc * xc, axis=-1, keepdims=True)
    return xc * jax.lax.rsqrt(v + EPS)


def _gelu(x):
    c = math.sqrt(2.0 / math.pi)
    t = jnp.tanh(x * (c + (c * 0.044715) * (x * x)))
    hx = 0.5 * x
    return hx + hx * t


def _dot(a, b):
    return jnp.dot(a, b, preferred_element_type=F32)


def _permute_cols(w_ref, r0, nr, c0):
    blk = [pltpu.bitcast(w_ref[pl.ds(r0, nr), c0 + b * 128:c0 + (b + 1) * 128], jnp.uint32)
           for b in range(NCB)]
    lane = jax.lax.broadcasted_iota(jnp.int32, blk[0].shape, 1)
    src = (lane & 3) * 32 + (lane & 28) + (lane >> 5)
    blk = [jnp.take_along_axis(x, src, axis=1) for x in blk]
    for t in range(3):
        sh = 4 << t
        low = (lane & sh) == 0
        for b in range(NCB):
            if b & (1 << t):
                continue
            lo, hi = blk[b], blk[b | (1 << t)]
            blk[b] = jnp.where(low, lo, pltpu.roll(hi, sh, 1))
            blk[b | (1 << t)] = jnp.where(low, pltpu.roll(lo, 128 - sh, 1), hi)
    for b in range(NCB):
        w_ref[pl.ds(r0, nr), c0 + b * 128:c0 + (b + 1) * 128] = pltpu.bitcast(blk[b], BF)


def _kernel(x_h, c_ref, wmod_h, wqkv_h, wo_h, w1_h, w2_h, w3_h, w4_h, out_h,
            xv, wmod, wqkv, wo, w1, w2, w3, w4, wo_tmp, mod, qbuf, kbuf, vbuf, obuf,
            xa, hb, h1, ostage, sems, osem):
    def cols(src, dst, c0, n):
        return src.at[:, pl.ds(c0, n)], dst.at[:, pl.ds(c0, n)]

    def rows(src, dst, r0, n):
        return src.at[pl.ds(r0, n)], dst.at[pl.ds(r0, n)]

    pairs = dict(
        wq=cols(wqkv_h, wqkv, 0, D), mod0=cols(wmod_h, wmod, 0, 2 * D), x0=rows(x_h, xv, 0, T),
        wk=cols(wqkv_h, wqkv, D, D), wv=cols(wqkv_h, wqkv, 2 * D, D),
        mod1=cols(wmod_h, wmod, 2 * D, 4 * D), wo=(wo_h, wo), w1=(w1_h, w1),
        x1=rows(x_h, xv, T, S - T), w2=(w2_h, w2), w3=(w3_h, w3), w4=(w4_h, w4))
    cp = {k: pltpu.make_async_copy(s_, d_, sems.at[n]) for n, (k, (s_, d_)) in enumerate(pairs.items())}

    def silu_c():
        cv = c_ref[...].astype(F32)
        s = (cv * jax.nn.sigmoid(cv)).astype(BF)
        return jnp.broadcast_to(s, (16, D))

    def perm(j):
        for r0 in range(0, D, 64):
            _permute_cols(wqkv, r0, 64, j * D)

    def a_ln(blk):
        x = xv[blk * T:(blk + 1) * T, :].astype(F32)
        return (_ln(x) * (1.0 + mod[1:2, :]) + mod[0:1, :]).astype(BF)

    def a_proj(blk, h, j):
        y = _dot(h, wqkv[:, j * D:(j + 1) * D])
        for b in range(NCB):
            yb = y[:, b * 128:(b + 1) * 128]
            if j == 0:
                qbuf[blk % 2, b] = yb * (DH ** -0.5)
            else:
                (kbuf, vbuf)[j - 1][b, HALO + blk * T:HALO + (blk + 1) * T, :] = yb

    def a_attn(blk, r0):
        first = blk == 0
        q = [qbuf[blk % 2, b, r0:r0 + RC, :] for b in range(NCB)]
        ls = []
        for w in range(W):
            o = HALO + blk * T + r0 - DIL * w
            acc = None
            for b in range(NCB):
                p = q[b] * kbuf[b, o:o + RC, :]
                acc = p if acc is None else acc + p
            acc = acc + pltpu.roll(acc, 64, 1)
            acc = acc + pltpu.roll(acc, 32, 1)
            if first and r0 < DIL * w:
                pos = jax.lax.broadcasted_iota(jnp.int32, acc.shape, 0) + r0
                acc = jnp.where(pos >= DIL * w, acc, -1e9)
            ls.append(acc)
        m = functools.reduce(jnp.maximum, ls)
        es = [jnp.exp(l - m) for l in ls]
        inv = 1.0 / functools.reduce(lambda a, b: a + b, es)
        ps = [e * inv for e in es]
        for b in range(NCB):
            acc = None
            for w in range(W):
                o = HALO + blk * T + r0 - DIL * w
                p = ps[w] * vbuf[b, o:o + RC, :]
                acc = p if acc is None else acc + p
            obuf[r0:r0 + RC, b * 128:(b + 1) * 128] = acc.astype(BF)

    def a_wo(slot):
        xn = xv[slot * T:(slot + 1) * T, :].astype(F32) + mod[2:3, :] * _dot(obuf[...], wo[...])
        h = _ln(xn) * (1.0 + mod[4:5, :]) + mod[3:4, :]
        r = HALO + slot * T
        xa[pl.ds(r, T), :] = xn
        hb[pl.ds(r, T), :] = h
        return _ln(h).astype(BF)

    def a_w1(slot, hn):
        g = _gelu(_dot(hn, w1[...]))
        r1 = 2 * HALO + slot * T
        for b in range(NCB):
            h1[b, pl.ds(r1, T), :] = g[:, b * 128:(b + 1) * 128]

    def b_head(blk, n):
        r = blk * T
        parts = []
        for b in range(NCB):
            sh = (1, -1, 2, -2)[b // 2]
            parts.append(h1[b, pl.ds(r + HALO - sh, n), :].astype(BF))
        hs = _dot(jnp.concatenate(parts, axis=1), w2[...])
        x1 = hb[pl.ds(r, n), :] + hs
        return x1, _ln(x1).astype(BF)

    def b_chunk(acc, ln1, f):
        g = _gelu(_dot(ln1, w3[:, f * FC:(f + 1) * FC])).astype(BF)
        return acc + _dot(g, w4[f * FC:(f + 1) * FC, :])

    def b_tail(blk, n, acc):
        r = blk * T
        y = xa[pl.ds(r, n), :] + mod[5:6, :] * acc
        ostage[pl.ds(r, n), :] = y.astype(BF)

    def out_copy(blk):
        lo = max(blk * T - HALO, 0)
        hi = S if blk == NB - 1 else (blk + 1) * T - HALO
        return pltpu.make_async_copy(ostage.at[pl.ds(lo + HALO, hi - lo)], out_h.at[pl.ds(lo, hi - lo)], osem.at[blk])

    nrc = T // RC

    def start(*names):
        for k in names:
            cp[k].start()

    start("wq", "mod0", "x0")
    xa[0:HALO, :] = jnp.zeros((HALO, D), F32)
    hb[0:HALO, :] = jnp.zeros((HALO, D), F32)
    for b in range(NCB):
        h1[b, 0:2 * HALO, :] = jnp.zeros((2 * HALO, 128), F32)
        h1[b, S + 2 * HALO:, :] = jnp.zeros((HALO, 128), F32)
        kbuf[b, 0:HALO, :] = jnp.zeros((HALO, 128), F32)
    sc = silu_c()
    cp["wq"].wait()
    start("wk")
    perm(0)
    cp["mod0"].wait()
    start("wv", "x1")
    for j in range(2):
        mod[j:j + 1, :] = _dot(sc, wmod[:, j * D:(j + 1) * D])[0:1, :]
    cp["x0"].wait()
    h = a_ln(0)
    cp["wk"].wait()
    start("wo", "mod1")
    a_proj(0, h, 0)
    perm(1)
    cp["wv"].wait()
    a_proj(0, h, 1)
    perm(2)
    a_proj(0, h, 2)
    for b in range(NCB):
        vbuf[b, 0:HALO, :] = jnp.broadcast_to(vbuf[b, HALO:HALO + 1, :], (HALO, 128))
    cp["x1"].wait()
    cp["wo"].wait()
    start("w1", "w2", "w3", "w4")
    h = a_ln(1)
    for b in range(NCB):
        wo_tmp[b] = wo[:, b * 128:(b + 1) * 128].astype(F32)
    for j in range(3):
        a_proj(1, h, j)
        for c in range(j * nrc // 3, (j + 1) * nrc // 3):
            a_attn(0, c * RC)
        for d in range(j * DH // 3, (j + 1) * DH // 3):
            rws = jnp.concatenate([wo_tmp[b, pl.ds(d, H, stride=DH), :] for b in range(NCB)], axis=1)
            wo[d * H:(d + 1) * H, :] = rws.astype(BF)
    cp["mod1"].wait()
    for j in range(2, 6):
        mod[j:j + 1, :] = _dot(sc, wmod[:, j * D:(j + 1) * D])[0:1, :]
    hn = a_wo(0)
    h = a_ln(2)
    cp["w1"].wait()
    a_w1(0, hn)
    for k in ("w2", "w3", "w4"):
        cp[k].wait()

    NA = 4
    for i in range(1, NB):
        x1, ln1 = b_head(i - 1, T)
        if i + 1 < NB:
            for j in range(3):
                a_proj(i + 1, h, j)
        acc = x1
        for f in range(NF):
            acc = b_chunk(acc, ln1, f)
            for c in range(f * nrc // NA, min((f + 1) * nrc // NA, nrc)):
                a_attn(i, c * RC)
            if f == NA - 1:
                hn = a_wo(i)
            if f == NA:
                a_w1(i, hn)
            if f == NA + 1 and i + 2 < NB:
                h = a_ln(i + 2)
        b_tail(i - 1, T, acc)
        out_copy(i - 1).start()

    n = T + HALO
    x1, ln1 = b_head(NB - 1, n)
    acc = x1
    for f in range(NF):
        acc = b_chunk(acc, ln1, f)
    b_tail(NB - 1, n, acc)
    out_copy(NB - 1).start()
    for blk in range(NB):
        out_copy(blk).wait()


@jax.jit
def pallas_adaLN_cond__sliding_local_dilated__mixer_s_mlp__prompt_kernel(
    A_x: jax.Array,
    A_wqkv: jax.Array,
    A_wo: jax.Array,
    B_x: jax.Array,
    B_w1: jax.Array,
    B_w2: jax.Array,
    B_w3: jax.Array,
    B_w4: jax.Array,
    c: jax.Array,
    w_mod: jax.Array,
):
    del B_x
    hbm = pl.BlockSpec(memory_space=pl.ANY)
    out = pl.pallas_call(
        _kernel,
        in_specs=[
            hbm,
            pl.BlockSpec(memory_space=pltpu.VMEM),
        ] + [hbm] * 7,
        out_specs=hbm,
        out_shape=jax.ShapeDtypeStruct((S, D), BF),
        scratch_shapes=[
            pltpu.VMEM((S, D), BF),
            pltpu.VMEM((D, 6 * D), BF),
            pltpu.VMEM((D, 3 * D), BF),
            pltpu.VMEM((D, D), BF),
            pltpu.VMEM((D, D), BF),
            pltpu.VMEM((D, D), BF),
            pltpu.VMEM((D, F), BF),
            pltpu.VMEM((F, D), BF),
            pltpu.VMEM((NCB, D, 128), F32),
            pltpu.VMEM((8, D), F32),
            pltpu.VMEM((2, NCB, T, 128), F32),
            pltpu.VMEM((NCB, S + HALO, 128), F32),
            pltpu.VMEM((NCB, S + HALO, 128), F32),
            pltpu.VMEM((T, D), BF),
            pltpu.VMEM((S + HALO, D), F32),
            pltpu.VMEM((S + HALO, D), F32),
            pltpu.VMEM((NCB, S + 3 * HALO, 128), F32),
            pltpu.VMEM((S + HALO, D), BF),
            pltpu.SemaphoreType.DMA((12,)),
            pltpu.SemaphoreType.DMA((NB,)),
        ],
        compiler_params=pltpu.CompilerParams(
            vmem_limit_bytes=120 * 1024 * 1024,
        ),
    )(A_x.reshape(S, D), c, w_mod, A_wqkv, A_wo, B_w1, B_w2, B_w3, B_w4)
    return out.reshape(1, S, D)
```

```python
import functools
import math

import jax
import jax.numpy as jnp
import jax.experimental.pallas as pl
import jax.experimental.pallas.tpu as pltpu

S, D, F = 2048, 1024, 3584
H, DH, W, DIL = 32, 32, 8, 2
T = 512
NB = S // T
HALO = 16
FC = 512
NF = F // FC
RC = 64
NCB = D // 128
BF, F32 = jnp.bfloat16, jnp.float32
EPS = 1e-5


def _ln(x):
    m = jnp.mean(x, axis=-1, keepdims=True)
    xc = x - m
    v = jnp.mean(xc * xc, axis=-1, keepdims=True)
    return xc * jax.lax.rsqrt(v + EPS)


def _gelu(x):
    c = math.sqrt(2.0 / math.pi)
    t = jnp.tanh(x * (c + (c * 0.044715) * (x * x)))
    hx = 0.5 * x
    return hx + hx * t


def _dot(a, b):
    return jnp.dot(a, b, preferred_element_type=F32)


def _permute_cols(w_ref, r0, nr, c0):
    blk = [pltpu.bitcast(w_ref[pl.ds(r0, nr), c0 + b * 128:c0 + (b + 1) * 128], jnp.uint32)
           for b in range(NCB)]
    lane = jax.lax.broadcasted_iota(jnp.int32, blk[0].shape, 1)
    src = (lane & 3) * 32 + (lane & 28) + (lane >> 5)
    blk = [jnp.take_along_axis(x, src, axis=1) for x in blk]
    for t in range(3):
        sh = 4 << t
        low = (lane & sh) == 0
        for b in range(NCB):
            if b & (1 << t):
                continue
            lo, hi = blk[b], blk[b | (1 << t)]
            blk[b] = jnp.where(low, lo, pltpu.roll(hi, sh, 1))
            blk[b | (1 << t)] = jnp.where(low, pltpu.roll(lo, 128 - sh, 1), hi)
    for b in range(NCB):
        w_ref[pl.ds(r0, nr), c0 + b * 128:c0 + (b + 1) * 128] = pltpu.bitcast(blk[b], BF)


def _kernel(x_h, c_ref, wmod_h, wqkv_h, wo_h, w1_h, w2_h, w3_h, w4_h, out_h,
            xv, wmod, wqkv, wo, w1, w2, w3, w4, wo_tmp, mod, qbuf, kbuf, vbuf, obuf,
            xa, hb, h1, ostage, sems, osem):
    def cols(src, dst, c0, n):
        return src.at[:, pl.ds(c0, n)], dst.at[:, pl.ds(c0, n)]

    def rows(src, dst, r0, n):
        return src.at[pl.ds(r0, n)], dst.at[pl.ds(r0, n)]

    pairs = dict(
        wq=cols(wqkv_h, wqkv, 0, D), mod0=cols(wmod_h, wmod, 0, 2 * D), x0=rows(x_h, xv, 0, T),
        wk=cols(wqkv_h, wqkv, D, D), wv=cols(wqkv_h, wqkv, 2 * D, D),
        mod1=cols(wmod_h, wmod, 2 * D, 4 * D), wo=(wo_h, wo), w1=(w1_h, w1),
        x1=rows(x_h, xv, T, S - T), w2=(w2_h, w2), w3=(w3_h, w3), w4=(w4_h, w4))
    cp = {k: pltpu.make_async_copy(s_, d_, sems.at[n]) for n, (k, (s_, d_)) in enumerate(pairs.items())}

    def silu_c():
        cv = c_ref[...].astype(F32)
        s = (cv * jax.nn.sigmoid(cv)).astype(BF)
        return jnp.broadcast_to(s, (16, D))

    def perm(j):
        for r0 in range(0, D, 64):
            _permute_cols(wqkv, r0, 64, j * D)

    def a_ln(blk):
        x = xv[blk * T:(blk + 1) * T, :].astype(F32)
        return (_ln(x) * (1.0 + mod[1:2, :]) + mod[0:1, :]).astype(BF)

    def a_proj(blk, h, j):
        y = _dot(h, wqkv[:, j * D:(j + 1) * D])
        for b in range(NCB):
            yb = y[:, b * 128:(b + 1) * 128]
            if j == 0:
                qbuf[blk % 2, b] = yb * (DH ** -0.5)
            else:
                (kbuf, vbuf)[j - 1][b, HALO + blk * T:HALO + (blk + 1) * T, :] = yb

    def a_attn(blk, r0):
        first = blk == 0
        q = [qbuf[blk % 2, b, r0:r0 + RC, :] for b in range(NCB)]
        ls = []
        for w in range(W):
            o = HALO + blk * T + r0 - DIL * w
            acc = None
            for b in range(NCB):
                p = q[b] * kbuf[b, o:o + RC, :]
                acc = p if acc is None else acc + p
            acc = acc + pltpu.roll(acc, 64, 1)
            acc = acc + pltpu.roll(acc, 32, 1)
            if first and r0 < DIL * w:
                pos = jax.lax.broadcasted_iota(jnp.int32, acc.shape, 0) + r0
                acc = jnp.where(pos >= DIL * w, acc, -1e9)
            ls.append(acc)
        m = functools.reduce(jnp.maximum, ls)
        es = [jnp.exp(l - m) for l in ls]
        inv = 1.0 / functools.reduce(lambda a, b: a + b, es)
        ps = [e * inv for e in es]
        for b in range(NCB):
            acc = None
            for w in range(W):
                o = HALO + blk * T + r0 - DIL * w
                p = ps[w] * vbuf[b, o:o + RC, :]
                acc = p if acc is None else acc + p
            obuf[r0:r0 + RC, b * 128:(b + 1) * 128] = acc.astype(BF)

    def a_wo(slot):
        xn = xv[slot * T:(slot + 1) * T, :].astype(F32) + mod[2:3, :] * _dot(obuf[...], wo[...])
        h = _ln(xn) * (1.0 + mod[4:5, :]) + mod[3:4, :]
        r = HALO + slot * T
        xa[pl.ds(r, T), :] = xn
        hb[pl.ds(r, T), :] = h
        return _ln(h).astype(BF)

    def a_w1(slot, hn):
        g = _gelu(_dot(hn, w1[...]))
        r1 = 2 * HALO + slot * T
        for b in range(NCB):
            h1[b, pl.ds(r1, T), :] = g[:, b * 128:(b + 1) * 128]

    def b_head(blk, n):
        r = blk * T
        parts = []
        for b in range(NCB):
            sh = (1, -1, 2, -2)[b // 2]
            parts.append(h1[b, pl.ds(r + HALO - sh, n), :].astype(BF))
        hs = _dot(jnp.concatenate(parts, axis=1), w2[...])
        x1 = hb[pl.ds(r, n), :] + hs
        return x1, _ln(x1).astype(BF)

    def b_chunk(acc, ln1, f):
        g = _gelu(_dot(ln1, w3[:, f * FC:(f + 1) * FC])).astype(BF)
        return acc + _dot(g, w4[f * FC:(f + 1) * FC, :])

    def b_tail(blk, n, acc):
        r = blk * T
        y = xa[pl.ds(r, n), :] + mod[5:6, :] * acc
        ostage[pl.ds(r, n), :] = y.astype(BF)

    def out_copy(blk):
        lo = max(blk * T - HALO, 0)
        hi = S if blk == NB - 1 else (blk + 1) * T - HALO
        return pltpu.make_async_copy(ostage.at[pl.ds(lo + HALO, hi - lo)], out_h.at[pl.ds(lo, hi - lo)], osem.at[blk])

    nrc = T // RC

    def start(*names):
        for k in names:
            cp[k].start()

    start("x0", "wq", "mod0")
    xa[0:HALO, :] = jnp.zeros((HALO, D), F32)
    hb[0:HALO, :] = jnp.zeros((HALO, D), F32)
    for b in range(NCB):
        h1[b, 0:2 * HALO, :] = jnp.zeros((2 * HALO, 128), F32)
        h1[b, S + 2 * HALO:, :] = jnp.zeros((HALO, 128), F32)
        kbuf[b, 0:HALO, :] = jnp.zeros((HALO, 128), F32)
    sc = silu_c()
    cp["x0"].wait()
    xn0 = _ln(xv[0:T, :].astype(F32))
    cp["wq"].wait()
    start("wk", "wv")
    perm(0)
    cp["mod0"].wait()
    for j in range(2):
        mod[j:j + 1, :] = _dot(sc, wmod[:, j * D:(j + 1) * D])[0:1, :]
    h = (xn0 * (1.0 + mod[1:2, :]) + mod[0:1, :]).astype(BF)
    cp["wk"].wait()
    start("x1", "wo", "mod1")
    a_proj(0, h, 0)
    perm(1)
    cp["wv"].wait()
    a_proj(0, h, 1)
    perm(2)
    cp["x1"].wait()
    cp["wo"].wait()
    start("w1", "w2", "w3", "w4")
    a_proj(0, h, 2)
    h = a_ln(1)
    for b in range(NCB):
        wo_tmp[b] = wo[:, b * 128:(b + 1) * 128].astype(F32)
    for b in range(NCB):
        vbuf[b, 0:HALO, :] = jnp.broadcast_to(vbuf[b, HALO:HALO + 1, :], (HALO, 128))
    for j in range(3):
        a_proj(1, h, j)
        for c in range(j * nrc // 3, (j + 1) * nrc // 3):
            a_attn(0, c * RC)
        for d in range(j * DH // 3, (j + 1) * DH // 3):
            rws = jnp.concatenate([wo_tmp[b, pl.ds(d, H, stride=DH), :] for b in range(NCB)], axis=1)
            wo[d * H:(d + 1) * H, :] = rws.astype(BF)
    cp["mod1"].wait()
    for j in range(2, 6):
        mod[j:j + 1, :] = _dot(sc, wmod[:, j * D:(j + 1) * D])[0:1, :]
    hn = a_wo(0)
    h = a_ln(2)
    cp["w1"].wait()
    a_w1(0, hn)
    for k in ("w2", "w3", "w4"):
        cp[k].wait()

    NA = 4
    for i in range(1, NB):
        x1, ln1 = b_head(i - 1, T)
        if i + 1 < NB:
            for j in range(3):
                a_proj(i + 1, h, j)
        acc = x1
        for f in range(NF):
            acc = b_chunk(acc, ln1, f)
            for c in range(f * nrc // NA, min((f + 1) * nrc // NA, nrc)):
                a_attn(i, c * RC)
            if f == NA - 1:
                hn = a_wo(i)
            if f == NA:
                a_w1(i, hn)
            if f == NA + 1 and i + 2 < NB:
                h = a_ln(i + 2)
        b_tail(i - 1, T, acc)
        out_copy(i - 1).start()

    n = T + HALO
    x1, ln1 = b_head(NB - 1, n)
    acc = x1
    for f in range(NF):
        acc = b_chunk(acc, ln1, f)
    b_tail(NB - 1, n, acc)
    out_copy(NB - 1).start()
    for blk in range(NB):
        out_copy(blk).wait()


@jax.jit
def pallas_adaLN_cond__sliding_local_dilated__mixer_s_mlp__prompt_kernel(
    A_x: jax.Array,
    A_wqkv: jax.Array,
    A_wo: jax.Array,
    B_x: jax.Array,
    B_w1: jax.Array,
    B_w2: jax.Array,
    B_w3: jax.Array,
    B_w4: jax.Array,
    c: jax.Array,
    w_mod: jax.Array,
):
    del B_x
    hbm = pl.BlockSpec(memory_space=pl.ANY)
    out = pl.pallas_call(
        _kernel,
        in_specs=[
            hbm,
            pl.BlockSpec(memory_space=pltpu.VMEM),
        ] + [hbm] * 7,
        out_specs=hbm,
        out_shape=jax.ShapeDtypeStruct((S, D), BF),
        scratch_shapes=[
            pltpu.VMEM((S, D), BF),
            pltpu.VMEM((D, 6 * D), BF),
            pltpu.VMEM((D, 3 * D), BF),
            pltpu.VMEM((D, D), BF),
            pltpu.VMEM((D, D), BF),
            pltpu.VMEM((D, D), BF),
            pltpu.VMEM((D, F), BF),
            pltpu.VMEM((F, D), BF),
            pltpu.VMEM((NCB, D, 128), F32),
            pltpu.VMEM((8, D), F32),
            pltpu.VMEM((2, NCB, T, 128), F32),
            pltpu.VMEM((NCB, S + HALO, 128), F32),
            pltpu.VMEM((NCB, S + HALO, 128), F32),
            pltpu.VMEM((T, D), BF),
            pltpu.VMEM((S + HALO, D), F32),
            pltpu.VMEM((S + HALO, D), F32),
            pltpu.VMEM((NCB, S + 3 * HALO, 128), F32),
            pltpu.VMEM((S + HALO, D), BF),
            pltpu.SemaphoreType.DMA((12,)),
            pltpu.SemaphoreType.DMA((NB,)),
        ],
        compiler_params=pltpu.CompilerParams(
            vmem_limit_bytes=120 * 1024 * 1024,
        ),
    )(A_x.reshape(S, D), c, w_mod, A_wqkv, A_wo, B_w1, B_w2, B_w3, B_w4)
    return out.reshape(1, S, D)
```
